```python
import os as _os
_os.environ.setdefault("JAX_PLATFORMS", "cpu")
import jax
import jax.numpy as jnp

def _softmax(x, axis=-1):
    return jax.nn.softmax(x, axis=axis)
def _gelu(x):
    return jax.nn.gelu(x, approximate=True)
def _silu(x):
    return jax.nn.silu(x)
def _sigmoid(x):
    return jax.nn.sigmoid(x)
def _layernorm(x, axis=-1, eps=1e-5):
    m = jnp.mean(x, axis=axis, keepdims=True)
    v = jnp.var(x, axis=axis, keepdims=True)
    return (x - m) / jnp.sqrt(v + eps)
def _scatter_add(tgt, idx, src, axis=0):
    return tgt.at[idx].add(src)
def _segment_sum(src, seg, n):
    return jax.ops.segment_sum(src, seg, n)
class _Rng:
    def __init__(self, key):
        self._k = key
    def _next(self):
        self._k, sub = jax.random.split(self._k)
        return sub
    def normal(self, shape):
        return jax.random.normal(self._next(), shape, dtype=jnp.bfloat16)
    def randint(self, lo, hi, shape):
        return jax.random.randint(self._next(), shape, lo, hi, dtype=jnp.int32)
    def uniform(self, shape, lo=0.0, hi=1.0):
        return jax.random.uniform(self._next(), shape, jnp.bfloat16, lo, hi)
    def permutation(self, n):
        return jax.random.permutation(self._next(), n)


kernel_name = 'concat_heads__sliding_block_cached__compressed_kv_cla__decode'

def setup_inputs():
    _rng = _Rng(jax.random.key(int.from_bytes(__import__("os").urandom(4), "little")))
    _w = (lambda a: (lambda t: t.astype(jnp.bfloat16) if jnp.issubdtype(t.dtype, jnp.floating) else t)(jnp.asarray(a)))
    def _A_setup():
        B, Sq, D = 1, 1, 512
        Hq, Hkv, Sk, Dh = 32, 32, 4096, 128
        assert Hq % Hkv == 0, (Hq, Hkv)
        return {
            "x": _w((lambda *s: _rng.normal(s) * 0.8)(B, Sq, D)),
            "k_cache": _w((lambda *s: _rng.normal(s) * 0.8)(B, Hkv, Sk, Dh)),
            "v_cache": _w((lambda *s: _rng.normal(s) * 0.05)(B, Hkv, Sk, Dh)),
            "wq": _w((lambda *s: _rng.normal(s) * 0.8)(D, Hq * Dh) * (D ** -0.5)),
            "wo": _w((lambda *s: _rng.normal(s) * 0.05)(Hq * Dh, D) * ((Hq * Dh) ** -0.5)),
        }
    _A_in = _A_setup()

    def _B_setup():
        B, H, Sq, Sk, D, M = 1, 32, 1, 4096, 128, 512
        Dc = 4 * D
        return {
            "x": _w((lambda *s: _rng.normal(s) * 1.6)(B, Sq, M)),
            "c_kv": _w((lambda *s: _rng.normal(s) * 0.1)(B, Sk, Dc)),
            "w_q": _w((lambda *s: _rng.normal(s) * 1.6)(M, H, D) * (M ** -0.5)),
            "w_uk": _w((lambda *s: _rng.normal(s) * 1.6)(Dc, H, D) * (Dc ** -0.5)),
            "w_uv": _w((lambda *s: _rng.normal(s) * 0.1)(Dc, H, D) * (Dc ** -0.5)),
            "w_o": _w((lambda *s: _rng.normal(s) * 0.1)(H, D, M) * ((H * D) ** -0.5)),
        }
    _B_in = _B_setup()

    return {
        "A_x": _A_in["x"],
        "A_k_cache": _A_in["k_cache"],
        "A_v_cache": _A_in["v_cache"],
        "A_wq": _A_in["wq"],
        "A_wo": _A_in["wo"],
        "B_x": _B_in["x"],
        "B_c_kv": _B_in["c_kv"],
        "B_w_q": _B_in["w_q"],
        "B_w_uk": _B_in["w_uk"],
        "B_w_uv": _B_in["w_uv"],
        "B_w_o": _B_in["w_o"],
    }

def reference(A_x, A_k_cache, A_v_cache, A_wq, A_wo, B_x, B_c_kv, B_w_q, B_w_uk, B_w_uv, B_w_o):
    def _A_ref(x, k_cache, v_cache, wq, wo):
        B, Sq, D = x.shape
        Hq, Dh = 32, 128
        Hkv, Sk = k_cache.shape[1], k_cache.shape[2]
        W = min(4096, max(256, Sk // 4))
        rep = Hq // Hkv
        q = (lambda x, *d: x.transpose(*d))((x @ wq).reshape(B, Sq, Hq, Dh), 0, 2, 1, 3)
        k = jnp.repeat(k_cache[:, :, Sk - W:, :], rep, axis=1)
        v = jnp.repeat(v_cache[:, :, Sk - W:, :], rep, axis=1)
        scores = jnp.einsum("bhqd,bhkd->bhqk", q, k) * (Dh ** -0.5)
        p = _softmax(scores, axis=-1)
        o = jnp.einsum("bhqk,bhkd->bhqd", p, v)
        return (lambda x, *d: x.transpose(*d))(o, 0, 2, 1, 3).reshape(B, Sq, Hq * Dh) @ wo

    def _B_ref(x, c_kv, w_q, w_uk, w_uv, w_o):
        B, Sq, M = x.shape[0], x.shape[1], x.shape[2]
        Sk = c_kv.shape[1]
        H, D = w_q.shape[1], w_q.shape[2]
        q = jnp.einsum("bqm,mhd->bhqd", x, w_q)
        k = jnp.einsum("bkc,chd->bhkd", c_kv, w_uk)
        v = jnp.einsum("bkc,chd->bhkd", c_kv, w_uv)
        scores = jnp.einsum("bhqd,bhkd->bhqk", q, k) * (D ** -0.5)
        off = Sk - Sq
        qi = jnp.arange(Sq)[:, None]
        kj = jnp.arange(Sk)[None, :]
        cmask = kj <= (qi + off)
        scores = jnp.where(cmask[None, None], scores, -1e9)
        p = _softmax(scores, axis=-1)
        ctx = jnp.einsum("bhqk,bhkd->bhqd", p, v)
        return jnp.einsum("bhqd,hdm->bqm", ctx, w_o)

    a = _A_ref(A_x, A_k_cache, A_v_cache, A_wq, A_wo)
    b = _B_ref(B_x, B_c_kv, B_w_q, B_w_uk, B_w_uv, B_w_o)
    return jnp.concatenate([a, b], axis=-1)
```

```python
import functools
import jax, jax.numpy as jnp, numpy as np
from jax import lax
from jax.experimental import pallas as pl
from jax.experimental.pallas import tpu as pltpu

bf = jnp.bfloat16
f32 = jnp.float32
H, DH, W, SK, DC, DM = 32, 128, 1024, 4096, 512, 512
NT = (((1,), (1,)), ((), ()))
NN = (((1,), (0,)), ((), ()))


def make(wo_chunks=(16, 8, 4, 2, 1, 1), u_diag=8, kchunk=512, u_head=2, skip=()):
    def kernel(ax_h, k_h, v_h, wq_h, wo_h, bx_h, c_h, bwq_h, uk_h, uv_h, bwo_h, o_ref,
               ax_v, bx_v, k_v, v_v, wq_v, wo_v, c_v, bwq_v, uk_v, uv_v, bwo_v,
               t_v, s_v, row_v, sems):
        cp = {}
        def mk(name, src, dst):
            cp[name] = pltpu.make_async_copy(src, dst, sems.at[len(cp)])
        mk("bwq", bwq_h, bwq_v)
        mk("bx", bx_h, bx_v)
        mk("ax", ax_h, ax_v)
        mk("uk", uk_h, uk_v)
        mk("c", c_h.at[0], c_v)
        mk("wq", wq_h, wq_v)
        mk("k0", k_h.at[0, pl.ds(0, 16), pl.ds(SK - W, W)], k_v.at[pl.ds(0, 16)])
        mk("k1", k_h.at[0, pl.ds(16, 16), pl.ds(SK - W, W)], k_v.at[pl.ds(16, 16)])
        mk("v0", v_h.at[0, pl.ds(0, 16), pl.ds(SK - W, W)], v_v.at[pl.ds(0, 16)])
        mk("v1", v_h.at[0, pl.ds(16, 16), pl.ds(SK - W, W)], v_v.at[pl.ds(16, 16)])
        mk("uv", uv_h, uv_v)
        mk("wo", wo_h, wo_v)
        h0 = 0
        for i, n in enumerate(wo_chunks):
            mk(f"bwo{i}", bwo_h.at[pl.ds(h0, n)], bwo_v.at[pl.ds(h0, n)])
            h0 += n
        for c in cp.values():
            c.start()

        scale = DH ** -0.5
        diag = (lax.broadcasted_iota(jnp.int32, (H, 128), 0)
                == lax.broadcasted_iota(jnp.int32, (H, 128), 1) % H)

        def slab_tile(w_v, j):
            return jnp.concatenate([w_v[g * 128 + j] for g in range(4)], axis=0)

        def headwise_matvec(w_v):
            def body(i, acc):
                j0 = pl.multiple_of(i * u_diag, u_diag)
                t = t_v[pl.ds(j0, u_diag), :]
                for u in range(u_diag):
                    l = jnp.where(diag, jnp.broadcast_to(t[u:u + 1, :], (H, 128)), 0.0).astype(bf)
                    acc = acc + lax.dot_general(l, slab_tile(w_v, j0 + u), NN, preferred_element_type=f32)
                return acc
            return lax.fori_loop(0, 128 // u_diag, body, jnp.zeros((H, 128), f32))

        cp["bx"].wait()
        xb = bx_v[0].astype(f32)
        xs = jnp.concatenate([jnp.broadcast_to(xb[:, g * 128:(g + 1) * 128], (H, 128)) for g in range(4)], axis=0)
        t_v[...] = xs.T
        cp["bwq"].wait()
        qb = headwise_matvec(bwq_v).astype(bf)

        cp["uk"].wait()
        def qabs_body(i, _):
            j0 = pl.multiple_of(i * u_diag, u_diag)
            rows = []
            for u in range(u_diag):
                r = lax.dot_general(qb, slab_tile(uk_v, j0 + u), NT, preferred_element_type=f32)
                rows.append(jnp.sum(jnp.where(diag, r, 0.0), axis=0, keepdims=True))
            t_v[pl.ds(j0, u_diag), :] = jnp.concatenate(rows, axis=0)
            return 0
        lax.fori_loop(0, 128 // u_diag, qabs_body, 0)
        tt = t_v[...].T
        qabs = jnp.concatenate([tt[g * H:(g + 1) * H, :] for g in range(4)], axis=1).astype(bf)

        cp["c"].wait()
        nk = SK // kchunk
        def sc_body(i, m):
            k0 = pl.multiple_of(i * kchunk, kchunk)
            s = lax.dot_general(qabs, c_v[pl.ds(k0, kchunk), :], NT, preferred_element_type=f32) * scale
            s_v[i] = s
            for t in range(kchunk // 128):
                m = jnp.maximum(m, s[:, t * 128:(t + 1) * 128])
            return m
        m = lax.fori_loop(0, nk, sc_body, jnp.full((H, 128), -jnp.inf, f32))
        m = jnp.max(m, axis=1, keepdims=True)
        def ctx_body(i, carry):
            l, acc = carry
            k0 = pl.multiple_of(i * kchunk, kchunk)
            p = jnp.exp(s_v[i] - m)
            for t in range(kchunk // 128):
                l = l + p[:, t * 128:(t + 1) * 128]
            acc = acc + lax.dot_general(p.astype(bf), c_v[pl.ds(k0, kchunk), :], NN, preferred_element_type=f32)
            return l, acc
        l, acc = lax.fori_loop(0, nk, ctx_body, (jnp.zeros((H, 128), f32), jnp.zeros((H, DC), f32)))
        ctxc = acc / jnp.sum(l, axis=1, keepdims=True)
        t_v[...] = jnp.concatenate([ctxc[:, g * 128:(g + 1) * 128] for g in range(4)], axis=0).T

        cp["ax"].wait()
        xa = jnp.broadcast_to(ax_v[0].astype(f32), (16, DM)).astype(bf)
        cp["wq"].wait()
        def qa_body(i, _):
            n0 = pl.multiple_of(i * 512, 512)
            r = lax.dot_general(xa, wq_v[:, pl.ds(n0, 512)], NN, preferred_element_type=f32)
            for t in range(4):
                row_v[pl.ds(i * 4 + t, 1), :] = r[0:1, t * 128:(t + 1) * 128]
            return 0
        lax.fori_loop(0, 8, qa_body, 0)
        qa = row_v[...].astype(bf)

        row16 = lax.broadcasted_iota(jnp.int32, (16, 128), 0)
        ps = []
        for g in range(2):
            cp[f"k{g}"].wait()
            qg = qa[g * 16:(g + 1) * 16]
            def s_body(i, s):
                for u in range(u_head):
                    hh = i * u_head + u
                    r = lax.dot_general(qg, k_v[g * 16 + hh], NT, preferred_element_type=f32)
                    sel = row16 == hh
                    s = jnp.concatenate([jnp.where(sel, r[:, t * 128:(t + 1) * 128], s[:, t * 128:(t + 1) * 128])
                                         for t in range(W // 128)], axis=1)
                return s
            s = lax.fori_loop(0, 16 // u_head, s_body, jnp.zeros((16, W), f32)) * scale
            e = jnp.exp(s - jnp.max(s, axis=1, keepdims=True))
            ps.append((e.astype(bf), jnp.sum(e, axis=1, keepdims=True)))
        for g in range(2):
            cp[f"v{g}"].wait()
            p, l = ps[g]
            def o_body(i, o):
                for u in range(u_head):
                    hh = i * u_head + u
                    r = lax.dot_general(p, v_v[g * 16 + hh], NN, preferred_element_type=f32)
                    o = jnp.where(row16 == hh, r, o)
                return o
            o = lax.fori_loop(0, 16 // u_head, o_body, jnp.zeros((16, 128), f32))
            row_v[pl.ds(g * 16, 16), :] = o / l

        cp["uv"].wait()
        ctx = headwise_matvec(uv_v)

        def proj(w_at, h0, n, acc, unroll):
            def body(i, acc):
                for u in range(unroll):
                    hh = h0 + i * unroll + u
                    lhs = jnp.broadcast_to(row_v[pl.ds(hh, 1), :], (16, 128)).astype(bf)
                    acc = acc + lax.dot_general(lhs, w_at(hh), NN, preferred_element_type=f32)
                return acc
            if n == unroll:
                return body(0, acc)
            return lax.fori_loop(0, n // unroll, body, acc)

        cp["wo"].wait()
        out_a = proj(lambda hh: wo_v[pl.ds(pl.multiple_of(hh * 128, 128), 128), :], 0, H, jnp.zeros((16, DM), f32), 4)
        o_ref[0, :, 0:DM] = out_a[0:1].astype(bf)
        row_v[...] = ctx
        acc = jnp.zeros((16, DM), f32)
        h0 = 0
        for i, n in enumerate(wo_chunks):
            cp[f"bwo{i}"].wait()
            acc = proj(lambda hh: bwo_v[hh], h0, n, acc, min(n, 4))
            h0 += n
        o_ref[0, :, DM:2 * DM] = acc[0:1].astype(bf)

    def fn(ax, k, v, wq, wo, bx, ckv, bwq, wuk, wuv, bwo):
        hbm = pl.BlockSpec(memory_space=pltpu.HBM)
        return pl.pallas_call(
            kernel,
            out_shape=jax.ShapeDtypeStruct((1, 1, 2 * DM), bf),
            in_specs=[hbm] * 11,
            out_specs=pl.BlockSpec(memory_space=pltpu.VMEM),
            scratch_shapes=[
                pltpu.VMEM((1, 1, DM), bf), pltpu.VMEM((1, 1, DM), bf),
                pltpu.VMEM((H, W, DH), bf), pltpu.VMEM((H, W, DH), bf),
                pltpu.VMEM((DM, H * DH), bf), pltpu.VMEM((H * DH, DM), bf),
                pltpu.VMEM((SK, DC), bf),
                pltpu.VMEM((DM, H, DH), bf), pltpu.VMEM((DC, H, DH), bf), pltpu.VMEM((DC, H, DH), bf),
                pltpu.VMEM((H, DH, DM), bf),
                pltpu.VMEM((128, 128), f32), pltpu.VMEM((SK // kchunk, H, kchunk), f32), pltpu.VMEM((H, DH), f32),
                pltpu.SemaphoreType.DMA((12 + len(wo_chunks),)),
            ],
            compiler_params=pltpu.CompilerParams(vmem_limit_bytes=100 * 1024 * 1024),
        )(ax, k, v, wq, wo, bx, ckv, bwq, wuk, wuv, bwo)
    return fn


@jax.jit
def pallas_concat_heads__sliding_block_cached__compressed_kv_cla__decode_kernel(
    A_x, A_k_cache, A_v_cache, A_wq, A_wo, B_x, B_c_kv, B_w_q, B_w_uk, B_w_uv, B_w_o,
):
    return make()(A_x, A_k_cache, A_v_cache, A_wq, A_wo, B_x, B_c_kv, B_w_q, B_w_uk, B_w_uv, B_w_o)
```

```python
import jax
import jax.numpy as jnp
from jax import lax
import jax.experimental.pallas as pl
import jax.experimental.pallas.tpu as pltpu

BF16 = jnp.bfloat16
F32 = jnp.float32

H = 32
DH = 128
DM = 512
DC = 512
SK = 4096
W = min(4096, max(256, SK // 4))
LANES = 128
GROUPS = LANES // H

NN = (((1,), (0,)), ((), ()))
NT = (((1,), (1,)), ((), ()))

TILE_UNROLL = 8
KCHUNK = 512
HEAD_UNROLL = 2
PROJ_UNROLL = 4

MXU_CHUNK_HEADS = (22, 6)
VPU_CHUNK_ROWS = (368, 112, 32)
MXU_HEADS = sum(MXU_CHUNK_HEADS)
assert sum(VPU_CHUNK_ROWS) == (H - MXU_HEADS) * DH
assert DM == DC == GROUPS * LANES


def _lane_tiles(x):
    return [x[:, t:t + LANES] for t in range(0, x.shape[1], LANES)]


def _kernel(ax_h, k_h, v_h, wq_h, wo_h, bx_h, c_h, bwq_h, uk_h, uv_h, bwo_h,
            o_ref,
            ax_v, k_v, v_v, wq_v, wo_v, bx_v, c_v, bwq_v, uk_v, uv_v, bwo_v,
            coef_v, score_v, head_v, col_v):
    window = pl.ds(SK - W, W)
    transfers = {
        "bwq": (bwq_h, bwq_v),
        "bx": (bx_h, bx_v),
        "ax": (ax_h, ax_v),
        "uk": (uk_h, uk_v),
        "c": (c_h.at[0], c_v),
        "wq": (wq_h, wq_v),
        "k": (k_h.at[0, :, window], k_v),
        "v": (v_h.at[0, :, window], v_v),
        "uv": (uv_h, uv_v),
        "wo": (wo_h, wo_v),
    }
    row = 0
    for i, n in enumerate([n * DH for n in MXU_CHUNK_HEADS] + list(VPU_CHUNK_ROWS)):
        transfers[f"bwo{i}"] = (bwo_h.at[pl.ds(row, n)], bwo_v.at[pl.ds(row, n)])
        row += n

    def body(sems):
        copies = {name: pltpu.make_async_copy(src, dst, sems.at[i])
                  for i, (name, (src, dst)) in enumerate(transfers.items())}
        for copy in copies.values():
            copy.start()

        scale = DH ** -0.5
        own_head = (lax.broadcasted_iota(jnp.int32, (H, LANES), 0)
                    == lax.broadcasted_iota(jnp.int32, (H, LANES), 1) % H)

        def tile(w_v, j):
            return jnp.concatenate([w_v[g * LANES + j] for g in range(GROUPS)], axis=0)

        def headwise_matvec(coef, w_v):
            coef_v[...] = jnp.concatenate(_lane_tiles(coef), axis=0).T

            def step(i, acc):
                j0 = pl.multiple_of(i * TILE_UNROLL, TILE_UNROLL)
                rows = coef_v[pl.ds(j0, TILE_UNROLL), :]
                for u in range(TILE_UNROLL):
                    lhs = jnp.where(own_head, jnp.broadcast_to(rows[u:u + 1], (H, LANES)), 0.0)
                    acc = acc + lax.dot_general(lhs.astype(BF16), tile(w_v, j0 + u), NN,
                                                preferred_element_type=F32)
                return acc

            return lambda: lax.fori_loop(0, LANES // TILE_UNROLL, step, jnp.zeros((H, DH), F32))

        copies["bx"].wait()
        run = headwise_matvec(jnp.broadcast_to(bx_v[0].astype(F32), (H, DM)), bwq_v)
        copies["bwq"].wait()
        q_b = run().astype(BF16)

        copies["uk"].wait()

        def absorb_step(i, carry):
            j0 = pl.multiple_of(i * TILE_UNROLL, TILE_UNROLL)
            rows = []
            for u in range(TILE_UNROLL):
                r = lax.dot_general(q_b, tile(uk_v, j0 + u), NT, preferred_element_type=F32)
                rows.append(jnp.sum(jnp.where(own_head, r, 0.0), axis=0, keepdims=True))
            coef_v[pl.ds(j0, TILE_UNROLL), :] = jnp.concatenate(rows, axis=0)
            return carry

        lax.fori_loop(0, LANES // TILE_UNROLL, absorb_step, 0)
        stacked = coef_v[...].T
        q_latent = jnp.concatenate([stacked[g * H:(g + 1) * H] for g in range(GROUPS)],
                                   axis=1).astype(BF16)

        copies["c"].wait()

        def score_step(i, m):
            k0 = pl.multiple_of(i * KCHUNK, KCHUNK)
            s = lax.dot_general(q_latent, c_v[pl.ds(k0, KCHUNK), :], NT,
                                preferred_element_type=F32) * scale
            key = k0 + lax.broadcasted_iota(jnp.int32, (H, KCHUNK), 1)
            s = jnp.where(key <= SK - 1, s, -1e9)
            score_v[i] = s
            for part in _lane_tiles(s):
                m = jnp.maximum(m, part)
            return m

        m = lax.fori_loop(0, SK // KCHUNK, score_step, jnp.full((H, LANES), -jnp.inf, F32))
        m = jnp.max(m, axis=1, keepdims=True)

        def context_step(i, carry):
            l, acc = carry
            k0 = pl.multiple_of(i * KCHUNK, KCHUNK)
            p = jnp.exp(score_v[i] - m)
            for part in _lane_tiles(p):
                l = l + part
            acc = acc + lax.dot_general(p.astype(BF16), c_v[pl.ds(k0, KCHUNK), :], NN,
                                        preferred_element_type=F32)
            return l, acc

        l, acc = lax.fori_loop(0, SK // KCHUNK, context_step,
                               (jnp.zeros((H, LANES), F32), jnp.zeros((H, DC), F32)))
        context_b = headwise_matvec(acc / jnp.sum(l, axis=1, keepdims=True), uv_v)

        copies["ax"].wait()
        x_a = jnp.broadcast_to(ax_v[0].astype(F32), (16, DM)).astype(BF16)
        copies["wq"].wait()

        def q_step(i, carry):
            n0 = pl.multiple_of(i * 4 * DH, 4 * DH)
            r = lax.dot_general(x_a, wq_v[:, pl.ds(n0, 4 * DH)], NN, preferred_element_type=F32)
            for t, part in enumerate(_lane_tiles(r[0:1])):
                head_v[pl.ds(i * 4 + t, 1), :] = part
            return carry

        lax.fori_loop(0, H // 4, q_step, 0)

        head16 = lax.broadcasted_iota(jnp.int32, (16, LANES), 0)
        copies["k"].wait()
        softmax_a = []
        for h0 in range(0, H, 16):
            q = head_v[pl.ds(h0, 16), :].astype(BF16)

            def qk_step(i, s):
                for u in range(HEAD_UNROLL):
                    h = i * HEAD_UNROLL + u
                    r = lax.dot_general(q, k_v[h0 + h], NT, preferred_element_type=F32)
                    s = jnp.concatenate([jnp.where(head16 == h, new, old) for new, old
                                         in zip(_lane_tiles(r), _lane_tiles(s))], axis=1)
                return s

            s = lax.fori_loop(0, 16 // HEAD_UNROLL, qk_step, jnp.zeros((16, W), F32)) * scale
            e = jnp.exp(s - jnp.max(s, axis=1, keepdims=True))
            softmax_a.append((e.astype(BF16), jnp.sum(e, axis=1, keepdims=True)))

        copies["v"].wait()
        for h0, (p, l) in zip(range(0, H, 16), softmax_a):

            def pv_step(i, o):
                for u in range(HEAD_UNROLL):
                    h = i * HEAD_UNROLL + u
                    r = lax.dot_general(p, v_v[h0 + h], NN, preferred_element_type=F32)
                    o = jnp.where(head16 == h, r, o)
                return o

            o = lax.fori_loop(0, 16 // HEAD_UNROLL, pv_step, jnp.zeros((16, DH), F32))
            head_v[pl.ds(h0, 16), :] = o / l

        copies["uv"].wait()
        ctx = context_b().astype(BF16).astype(F32)
        for h in range(MXU_HEADS, H):
            col_v[pl.ds((h - MXU_HEADS) * DH, DH), :] = jnp.broadcast_to(ctx[h:h + 1], (LANES, DH)).T

        def project(w_v, h0, n, acc):
            def one(h, acc):
                r0 = h * DH if isinstance(h, int) else pl.multiple_of(h * DH, DH)
                lhs = jnp.broadcast_to(head_v[pl.ds(h, 1), :], (16, DH)).astype(BF16)
                return acc + lax.dot_general(lhs, w_v[pl.ds(r0, DH), :], NN,
                                             preferred_element_type=F32)

            def step(i, acc):
                for u in range(PROJ_UNROLL):
                    acc = one(h0 + i * PROJ_UNROLL + u, acc)
                return acc

            steps = n // PROJ_UNROLL if n >= 2 * PROJ_UNROLL else 0
            if steps:
                acc = lax.fori_loop(0, steps, step, acc)
            for h in range(h0 + steps * PROJ_UNROLL, h0 + n):
                acc = one(h, acc)
            return acc

        copies["wo"].wait()
        out_a = project(wo_v, 0, H, jnp.zeros((16, DM), F32))
        o_ref[0, :, 0:DM] = out_a[0:1].astype(BF16)

        head_v[...] = ctx
        acc = jnp.zeros((16, DM), F32)
        h0 = 0
        for i, n in enumerate(MXU_CHUNK_HEADS):
            copies[f"bwo{i}"].wait()
            acc = project(bwo_v, h0, n, acc)
            h0 += n
        acc = jnp.where(lax.broadcasted_iota(jnp.int32, (8, DM), 0) == 0, acc[0:8], 0.0)
        r0 = MXU_HEADS * DH
        for i, n in enumerate(VPU_CHUNK_ROWS):
            copies[f"bwo{len(MXU_CHUNK_HEADS) + i}"].wait()
            for r in range(r0, r0 + n, 16):
                col = col_v[pl.ds(r - MXU_HEADS * DH, 16), :]
                prod = (bwo_v[pl.ds(r, 16), :].astype(F32)
                        * jnp.concatenate([col] * (DM // LANES), axis=1))
                acc = acc + (prod[0:8] + prod[8:16])
            r0 += n
        o_ref[0, :, DM:2 * DM] = jnp.sum(acc, axis=0, keepdims=True).astype(BF16)

    pl.run_scoped(body, pltpu.SemaphoreType.DMA((len(transfers),)))


@jax.jit
def pallas_concat_heads__sliding_block_cached__compressed_kv_cla__decode_kernel(
    A_x: jax.Array,
    A_k_cache: jax.Array,
    A_v_cache: jax.Array,
    A_wq: jax.Array,
    A_wo: jax.Array,
    B_x: jax.Array,
    B_c_kv: jax.Array,
    B_w_q: jax.Array,
    B_w_uk: jax.Array,
    B_w_uv: jax.Array,
    B_w_o: jax.Array,
):
    assert A_x.shape == B_x.shape == (1, 1, DM)
    assert A_k_cache.shape == A_v_cache.shape == (1, H, SK, DH)
    assert B_c_kv.shape == (1, SK, DC)
    operands = (A_x, A_k_cache, A_v_cache, A_wq, A_wo,
                B_x, B_c_kv, B_w_q, B_w_uk, B_w_uv, B_w_o.reshape(H * DH, DM))
    return pl.pallas_call(
        _kernel,
        out_shape=jax.ShapeDtypeStruct((1, 1, 2 * DM), BF16),
        in_specs=[pl.BlockSpec(memory_space=pltpu.HBM)] * len(operands),
        out_specs=pl.BlockSpec(memory_space=pltpu.VMEM),
        scratch_shapes=[
            pltpu.VMEM((1, 1, DM), BF16),
            pltpu.VMEM((H, W, DH), BF16),
            pltpu.VMEM((H, W, DH), BF16),
            pltpu.VMEM((DM, H * DH), BF16),
            pltpu.VMEM((H * DH, DM), BF16),
            pltpu.VMEM((1, 1, DM), BF16),
            pltpu.VMEM((SK, DC), BF16),
            pltpu.VMEM((DM, H, DH), BF16),
            pltpu.VMEM((DC, H, DH), BF16),
            pltpu.VMEM((DC, H, DH), BF16),
            pltpu.VMEM((H * DH, DM), BF16),
            pltpu.VMEM((LANES, LANES), F32),
            pltpu.VMEM((SK // KCHUNK, H, KCHUNK), F32),
            pltpu.VMEM((H, DH), F32),
            pltpu.VMEM(((H - MXU_HEADS) * DH, LANES), F32),
        ],
        compiler_params=pltpu.CompilerParams(vmem_limit_bytes=64 * 1024 * 1024),
    )(*operands)
```

```python
import jax
import jax.numpy as jnp
from jax import lax
import jax.experimental.pallas as pl
import jax.experimental.pallas.tpu as pltpu

BF16 = jnp.bfloat16
F32 = jnp.float32

H = 32
DH = 128
DM = 512
DC = 512
SK = 4096
W = min(4096, max(256, SK // 4))
LANES = 128
GROUPS = LANES // H

NN = (((1,), (0,)), ((), ()))
NT = (((1,), (1,)), ((), ()))

TILE_UNROLL = 8
KCHUNK = 512
HEAD_UNROLL = 2
PROJ_UNROLL = 4

MXU_CHUNK_HEADS = (22, 6)
VPU_CHUNK_ROWS = (368, 112, 32)
MXU_HEADS = sum(MXU_CHUNK_HEADS)
assert sum(VPU_CHUNK_ROWS) == (H - MXU_HEADS) * DH
assert DM == DC == GROUPS * LANES


def _lane_tiles(x):
    return [x[:, t:t + LANES] for t in range(0, x.shape[1], LANES)]


def _kernel(ax_h, k_h, v_h, wq_h, wo_h, bx_h, c_h, bwq_h, uk_h, uv_h, bwo_h,
            o_ref,
            ax_v, k_v, v_v, wq_v, wo_v, bx_v, c_v, bwq_v, uk_v, uv_v, bwo_v,
            coef_v, score_v, head_v, col_v):
    window = pl.ds(SK - W, W)
    transfers = {
        "bwq": (bwq_h, bwq_v),
        "bx": (bx_h, bx_v),
        "ax": (ax_h, ax_v),
        "uk": (uk_h, uk_v),
        "c": (c_h.at[0], c_v),
        "wq": (wq_h, wq_v),
        "k": (k_h.at[0, :, window], k_v),
        "v": (v_h.at[0, :, window], v_v),
        "uv": (uv_h, uv_v),
        "wo": (wo_h, wo_v),
    }
    row = 0
    for i, n in enumerate([n * DH for n in MXU_CHUNK_HEADS] + list(VPU_CHUNK_ROWS)):
        transfers[f"bwo{i}"] = (bwo_h.at[pl.ds(row, n)], bwo_v.at[pl.ds(row, n)])
        row += n

    def body(sems):
        copies = {name: pltpu.make_async_copy(src, dst, sems.at[i])
                  for i, (name, (src, dst)) in enumerate(transfers.items())}
        for copy in copies.values():
            copy.start()

        scale = DH ** -0.5
        own_head = (lax.broadcasted_iota(jnp.int32, (H, LANES), 0)
                    == lax.broadcasted_iota(jnp.int32, (H, LANES), 1) % H)

        def tile(w_v, j):
            return jnp.concatenate([w_v[g * LANES + j] for g in range(GROUPS)], axis=0)

        def set_coef(coef):
            coef_v[...] = jnp.concatenate(_lane_tiles(coef), axis=0).T

        def headwise_matvec(w_v):
            def step(i, acc):
                j0 = pl.multiple_of(i * TILE_UNROLL, TILE_UNROLL)
                rows = coef_v[pl.ds(j0, TILE_UNROLL), :]
                for u in range(TILE_UNROLL):
                    lhs = jnp.where(own_head, jnp.broadcast_to(rows[u:u + 1], (H, LANES)), 0.0)
                    acc = acc + lax.dot_general(lhs.astype(BF16), tile(w_v, j0 + u), NN,
                                                preferred_element_type=F32)
                return acc

            return lax.fori_loop(0, LANES // TILE_UNROLL, step, jnp.zeros((H, DH), F32))

        copies["bx"].wait()
        set_coef(jnp.broadcast_to(bx_v[0].astype(F32), (H, DM)))
        copies["bwq"].wait()
        q_b = headwise_matvec(bwq_v).astype(BF16)

        copies["uk"].wait()

        def absorb_step(i, carry):
            j0 = pl.multiple_of(i * TILE_UNROLL, TILE_UNROLL)
            rows = []
            for u in range(TILE_UNROLL):
                r = lax.dot_general(q_b, tile(uk_v, j0 + u), NT, preferred_element_type=F32)
                rows.append(jnp.sum(jnp.where(own_head, r, 0.0), axis=0, keepdims=True))
            coef_v[pl.ds(j0, TILE_UNROLL), :] = jnp.concatenate(rows, axis=0)
            return carry

        lax.fori_loop(0, LANES // TILE_UNROLL, absorb_step, 0)
        stacked = coef_v[...].T
        q_latent = jnp.concatenate([stacked[g * H:(g + 1) * H] for g in range(GROUPS)],
                                   axis=1).astype(BF16)

        copies["c"].wait()

        def score_step(i, m):
            k0 = pl.multiple_of(i * KCHUNK, KCHUNK)
            s = lax.dot_general(q_latent, c_v[pl.ds(k0, KCHUNK), :], NT,
                                preferred_element_type=F32) * scale
            key = k0 + lax.broadcasted_iota(jnp.int32, (H, KCHUNK), 1)
            s = jnp.where(key <= SK - 1, s, -1e9)
            score_v[i] = s
            for part in _lane_tiles(s):
                m = jnp.maximum(m, part)
            return m

        m = lax.fori_loop(0, SK // KCHUNK, score_step, jnp.full((H, LANES), -jnp.inf, F32))
        m = jnp.max(m, axis=1, keepdims=True)

        def context_step(i, carry):
            l, acc = carry
            k0 = pl.multiple_of(i * KCHUNK, KCHUNK)
            p = jnp.exp(score_v[i] - m)
            for part in _lane_tiles(p):
                l = l + part
            acc = acc + lax.dot_general(p.astype(BF16), c_v[pl.ds(k0, KCHUNK), :], NN,
                                        preferred_element_type=F32)
            return l, acc

        l, acc = lax.fori_loop(0, SK // KCHUNK, context_step,
                               (jnp.zeros((H, LANES), F32), jnp.zeros((H, DC), F32)))
        set_coef(acc / jnp.sum(l, axis=1, keepdims=True))

        copies["ax"].wait()
        x_a = jnp.broadcast_to(ax_v[0].astype(F32), (16, DM)).astype(BF16)
        copies["wq"].wait()

        def q_step(i, carry):
            n0 = pl.multiple_of(i * 4 * DH, 4 * DH)
            r = lax.dot_general(x_a, wq_v[:, pl.ds(n0, 4 * DH)], NN, preferred_element_type=F32)
            for t, part in enumerate(_lane_tiles(r[0:1])):
                head_v[pl.ds(i * 4 + t, 1), :] = part
            return carry

        lax.fori_loop(0, H // 4, q_step, 0)

        head16 = lax.broadcasted_iota(jnp.int32, (16, LANES), 0)
        copies["k"].wait()
        softmax_a = []
        for h0 in range(0, H, 16):
            q = head_v[pl.ds(h0, 16), :].astype(BF16)

            def qk_step(i, s):
                for u in range(HEAD_UNROLL):
                    h = i * HEAD_UNROLL + u
                    r = lax.dot_general(q, k_v[h0 + h], NT, preferred_element_type=F32)
                    s = jnp.concatenate([jnp.where(head16 == h, new, old) for new, old
                                         in zip(_lane_tiles(r), _lane_tiles(s))], axis=1)
                return s

            s = lax.fori_loop(0, 16 // HEAD_UNROLL, qk_step, jnp.zeros((16, W), F32)) * scale
            e = jnp.exp(s - jnp.max(s, axis=1, keepdims=True))
            softmax_a.append((e.astype(BF16), jnp.sum(e, axis=1, keepdims=True)))

        copies["v"].wait()
        for h0, (p, l) in zip(range(0, H, 16), softmax_a):

            def pv_step(i, o):
                for u in range(HEAD_UNROLL):
                    h = i * HEAD_UNROLL + u
                    r = lax.dot_general(p, v_v[h0 + h], NN, preferred_element_type=F32)
                    o = jnp.where(head16 == h, r, o)
                return o

            o = lax.fori_loop(0, 16 // HEAD_UNROLL, pv_step, jnp.zeros((16, DH), F32))
            head_v[pl.ds(h0, 16), :] = o / l

        copies["uv"].wait()
        ctx = headwise_matvec(uv_v).astype(BF16).astype(F32)
        for h in range(MXU_HEADS, H):
            col_v[pl.ds((h - MXU_HEADS) * DH, DH), :] = jnp.broadcast_to(ctx[h:h + 1], (LANES, DH)).T

        def project(w_v, h0, n, acc):
            def one(h, acc):
                r0 = h * DH if isinstance(h, int) else pl.multiple_of(h * DH, DH)
                lhs = jnp.broadcast_to(head_v[pl.ds(h, 1), :], (16, DH)).astype(BF16)
                return acc + lax.dot_general(lhs, w_v[pl.ds(r0, DH), :], NN,
                                             preferred_element_type=F32)

            def step(i, acc):
                for u in range(PROJ_UNROLL):
                    acc = one(h0 + i * PROJ_UNROLL + u, acc)
                return acc

            steps = n // PROJ_UNROLL if n >= 2 * PROJ_UNROLL else 0
            if steps:
                acc = lax.fori_loop(0, steps, step, acc)
            for h in range(h0 + steps * PROJ_UNROLL, h0 + n):
                acc = one(h, acc)
            return acc

        copies["wo"].wait()
        out_a = project(wo_v, 0, H, jnp.zeros((16, DM), F32))
        o_ref[0, :, 0:DM] = out_a[0:1].astype(BF16)

        head_v[...] = ctx
        acc = jnp.zeros((16, DM), F32)
        h0 = 0
        for i, n in enumerate(MXU_CHUNK_HEADS):
            copies[f"bwo{i}"].wait()
            acc = project(bwo_v, h0, n, acc)
            h0 += n
        acc = jnp.where(lax.broadcasted_iota(jnp.int32, (8, DM), 0) == 0, acc[0:8], 0.0)
        r0 = MXU_HEADS * DH
        for i, n in enumerate(VPU_CHUNK_ROWS):
            copies[f"bwo{len(MXU_CHUNK_HEADS) + i}"].wait()
            for r in range(r0, r0 + n, 16):
                col = col_v[pl.ds(r - MXU_HEADS * DH, 16), :]
                prod = (bwo_v[pl.ds(r, 16), :].astype(F32)
                        * jnp.concatenate([col] * (DM // LANES), axis=1))
                acc = acc + (prod[0:8] + prod[8:16])
            r0 += n
        o_ref[0, :, DM:2 * DM] = jnp.sum(acc, axis=0, keepdims=True).astype(BF16)

    pl.run_scoped(body, pltpu.SemaphoreType.DMA((len(transfers),)))


@jax.jit
def pallas_concat_heads__sliding_block_cached__compressed_kv_cla__decode_kernel(
    A_x: jax.Array,
    A_k_cache: jax.Array,
    A_v_cache: jax.Array,
    A_wq: jax.Array,
    A_wo: jax.Array,
    B_x: jax.Array,
    B_c_kv: jax.Array,
    B_w_q: jax.Array,
    B_w_uk: jax.Array,
    B_w_uv: jax.Array,
    B_w_o: jax.Array,
):
    assert A_x.shape == B_x.shape == (1, 1, DM)
    assert A_k_cache.shape == A_v_cache.shape == (1, H, SK, DH)
    assert B_c_kv.shape == (1, SK, DC)
    operands = (A_x, A_k_cache, A_v_cache, A_wq, A_wo,
                B_x, B_c_kv, B_w_q, B_w_uk, B_w_uv, B_w_o.reshape(H * DH, DM))
    return pl.pallas_call(
        _kernel,
        out_shape=jax.ShapeDtypeStruct((1, 1, 2 * DM), BF16),
        in_specs=[pl.BlockSpec(memory_space=pltpu.HBM)] * len(operands),
        out_specs=pl.BlockSpec(memory_space=pltpu.VMEM),
        scratch_shapes=[
            pltpu.VMEM((1, 1, DM), BF16),
            pltpu.VMEM((H, W, DH), BF16),
            pltpu.VMEM((H, W, DH), BF16),
            pltpu.VMEM((DM, H * DH), BF16),
            pltpu.VMEM((H * DH, DM), BF16),
            pltpu.VMEM((1, 1, DM), BF16),
            pltpu.VMEM((SK, DC), BF16),
            pltpu.VMEM((DM, H, DH), BF16),
            pltpu.VMEM((DC, H, DH), BF16),
            pltpu.VMEM((DC, H, DH), BF16),
            pltpu.VMEM((H * DH, DM), BF16),
            pltpu.VMEM((LANES, LANES), F32),
            pltpu.VMEM((SK // KCHUNK, H, KCHUNK), F32),
            pltpu.VMEM((H, DH), F32),
            pltpu.VMEM(((H - MXU_HEADS) * DH, LANES), F32),
        ],
        compiler_params=pltpu.CompilerParams(vmem_limit_bytes=64 * 1024 * 1024),
    )(*operands)
```
